```python
import os as _os
_os.environ.setdefault("JAX_PLATFORMS", "cpu")
import jax
import jax.numpy as jnp

def _softmax(x, axis=-1):
    return jax.nn.softmax(x, axis=axis)
def _gelu(x):
    return jax.nn.gelu(x, approximate=True)
def _silu(x):
    return jax.nn.silu(x)
def _sigmoid(x):
    return jax.nn.sigmoid(x)
def _layernorm(x, axis=-1, eps=1e-5):
    m = jnp.mean(x, axis=axis, keepdims=True)
    v = jnp.var(x, axis=axis, keepdims=True)
    return (x - m) / jnp.sqrt(v + eps)
def _scatter_add(tgt, idx, src, axis=0):
    return tgt.at[idx].add(src)
def _segment_sum(src, seg, n):
    return jax.ops.segment_sum(src, seg, n)
class _Rng:
    def __init__(self, key):
        self._k = key
    def _next(self):
        self._k, sub = jax.random.split(self._k)
        return sub
    def normal(self, shape):
        return jax.random.normal(self._next(), shape, dtype=jnp.bfloat16)
    def randint(self, lo, hi, shape):
        return jax.random.randint(self._next(), shape, lo, hi, dtype=jnp.int32)
    def uniform(self, shape, lo=0.0, hi=1.0):
        return jax.random.uniform(self._next(), shape, jnp.bfloat16, lo, hi)
    def permutation(self, n):
        return jax.random.permutation(self._next(), n)


kernel_name = 'gated_mix__sliding_block_cached__swiglu_ffn__decode'

def setup_inputs():
    _rng = _Rng(jax.random.key(int.from_bytes(__import__("os").urandom(4), "little")))
    _w = (lambda a: (lambda t: t.astype(jnp.bfloat16) if jnp.issubdtype(t.dtype, jnp.floating) else t)(jnp.asarray(a)))
    def _A_setup():
        B, Sq, D = 1, 1, 512
        Hq, Hkv, Sk, Dh = 32, 32, 32768, 128
        assert Hq % Hkv == 0, (Hq, Hkv)
        return {
            "x": _w((lambda *s: _rng.normal(s) * 0.05)(B, Sq, D)),
            "k_cache": _w((lambda *s: _rng.normal(s) * 3.2)(B, Hkv, Sk, Dh)),
            "v_cache": _w((lambda *s: _rng.normal(s) * 1.6)(B, Hkv, Sk, Dh)),
            "wq": _w((lambda *s: _rng.normal(s) * 3.2)(D, Hq * Dh) * (D ** -0.5)),
            "wo": _w((lambda *s: _rng.normal(s) * 1.6)(Hq * Dh, D) * ((Hq * Dh) ** -0.5)),
        }
    _A_in = _A_setup()

    def _B_setup():
        B, S, D, F = 1, 1, 512, 1376
        return {
            "x": _w((lambda *s: _rng.normal(s) * 0.05)(B, S, D)),
            "w_gate": _w((lambda *s: _rng.normal(s) * 0.1)(D, F)),
            "w_up": _w((lambda *s: _rng.normal(s) * 0.1)(D, F)),
            "w_down": _w((lambda *s: _rng.normal(s) * 0.1)(F, D)),
        }
    _B_in = _B_setup()

    return {
        "A_x": _A_in["x"],
        "A_k_cache": _A_in["k_cache"],
        "A_v_cache": _A_in["v_cache"],
        "A_wq": _A_in["wq"],
        "A_wo": _A_in["wo"],
        "B_x": _B_in["x"],
        "B_w_gate": _B_in["w_gate"],
        "B_w_up": _B_in["w_up"],
        "B_w_down": _B_in["w_down"],
        "gate_w": _w((lambda *s: _rng.normal(s) * 0.05)(512) * 16.0),
    }

def reference(A_x, A_k_cache, A_v_cache, A_wq, A_wo, B_x, B_w_gate, B_w_up, B_w_down, gate_w):
    def _A_ref(x, k_cache, v_cache, wq, wo):
        B, Sq, D = x.shape
        Hq, Dh = 32, 128
        Hkv, Sk = k_cache.shape[1], k_cache.shape[2]
        W = min(4096, max(256, Sk // 4))
        rep = Hq // Hkv
        q = (lambda x, *d: x.transpose(*d))((x @ wq).reshape(B, Sq, Hq, Dh), 0, 2, 1, 3)
        k = jnp.repeat(k_cache[:, :, Sk - W:, :], rep, axis=1)
        v = jnp.repeat(v_cache[:, :, Sk - W:, :], rep, axis=1)
        scores = jnp.einsum("bhqd,bhkd->bhqk", q, k) * (Dh ** -0.5)
        p = _softmax(scores, axis=-1)
        o = jnp.einsum("bhqk,bhkd->bhqd", p, v)
        return (lambda x, *d: x.transpose(*d))(o, 0, 2, 1, 3).reshape(B, Sq, Hq * Dh) @ wo

    def _B_ref(x, w_gate, w_up, w_down):
        g = _silu(x @ w_gate)
        u = x @ w_up
        return (g * u) @ w_down

    x = A_x
    g = _sigmoid((x * gate_w).sum(-1, keepdims=True))
    a = _A_ref(x, A_k_cache, A_v_cache, A_wq, A_wo)
    b = _B_ref(x, B_w_gate, B_w_up, B_w_down)
    return g * a + (1 - g) * b
```

```python
import functools
import jax
import jax.numpy as jnp
from jax import lax
import jax.experimental.pallas as pl
import jax.experimental.pallas.tpu as pltpu

def build(NH=4, ROWS=32, CR=512, G=3, nobc=True, FFN_AT=48, WD_SPLIT=(1024, 1376), compute=True):
  def kernel_fn(A_x, A_k_cache, A_v_cache, A_wq, A_wo, B_x, B_w_gate, B_w_up, B_w_down, gate_w):
    B, Sq, D = A_x.shape
    H, Sk, Dh = A_k_cache.shape[1], A_k_cache.shape[2], A_k_cache.shape[3]
    F = B_w_gate.shape[1]
    W = min(4096, max(256, Sk // 4))
    scale = Dh ** -0.5
    NC = W // CR
    NG = H // NH
    NR = NG * NC
    ND = CR // ROWS
    S = G + 1
    GW = NH * Dh
    WR = 32
    NWQ = D // WR
    NWO = GW // WR
    assert NWQ % NC == 0 and NWO % NC == 0
    WQ_PER, WO_PER = NWQ // NC, NWO // NC
    NF = F // WR
    assert F % WR == 0 and D == GW
    f32, bf16 = jnp.float32, jnp.bfloat16
    NT = (((1,), (1,)), ((), ()))

    def kernel(x_hbm, gw_hbm, k_hbm, v_hbm, wq_hbm, wo_hbm, wg_hbm, wu_hbm, wd_hbm, o_ref,
               kv, x_v, gw_v, wq_v, wo_v, wg_v, wu_v, wd_v, q_s, m_s, l_s, acc_s, out_s, hid_s,
               kv_sem, wq_sem, wo_sem, misc_sem):
        def kv_dma(r, which, j, pr):
            g = r // NC
            c = r % NC
            slot = r % S
            src = (k_hbm, v_hbm)[which]
            pltpu.make_async_copy(
                src.at[0, pl.ds(g * NH, NH), pl.ds(Sk - W + c * CR + j * ROWS, ROWS), :],
                kv.at[slot, which, :, pl.ds(j * ROWS, ROWS), :], kv_sem.at[slot]).start(priority=pr)

        def wq_dma(g, i, pr):
            pltpu.make_async_copy(wq_hbm.at[pl.ds(i * WR, WR), pl.ds(g * GW, GW)],
                                  wq_v.at[g, pl.ds(i * WR, WR), :], wq_sem.at[g]).start(priority=pr)

        def wo_dma(g, i, pr):
            pltpu.make_async_copy(wo_hbm.at[pl.ds(g * GW + i * WR, WR), :],
                                  wo_v.at[g, pl.ds(i * WR, WR), :], wo_sem.at[g]).start(priority=pr)

        def rows_dma(src, dst, i, sem, pr):
            pltpu.make_async_copy(src.at[pl.ds(i * WR, WR), :], dst.at[pl.ds(i * WR, WR), :], sem).start(priority=pr)

        def issue_round(r):
            g = r // NC
            c = r % NC
            half = ND // 4
            for j in range(ND):
                kv_dma(r, 0, j, 0)
                kv_dma(r, 1, j, 1)
                if j == half:
                    for i in range(WO_PER):
                        wo_dma(g, c * WO_PER + i, i % 2)
                if j == 2 * half:
                    @pl.when(g + 1 < NG)
                    def _():
                        for i in range(WQ_PER):
                            wq_dma(g + 1, c * WQ_PER + i, i % 2)
                if j == 3 * half:
                    @pl.when(r < NF)
                    def _():
                        rows_dma(wg_hbm, wg_v, r, misc_sem.at[2], 0)
                        rows_dma(wu_hbm, wu_v, r, misc_sem.at[3], 1)

        def wait_all(buf, sem):
            pltpu.make_async_copy(buf, buf, sem).wait()

        cx = pltpu.make_async_copy(x_hbm, x_v, misc_sem.at[0])
        cg = pltpu.make_async_copy(gw_hbm, gw_v, misc_sem.at[1])
        cx.start()
        cg.start()
        for i in range(NWQ):
            wq_dma(0, i, i % 2)

        def pro(r, carry):
            issue_round(r)
            return carry
        lax.fori_loop(0, G, pro, 0)

        cx.wait()
        out_s[...] = jnp.zeros_like(out_s)
        row = lax.broadcasted_iota(jnp.int32, (8, GW), 0)
        blk = lax.broadcasted_iota(jnp.int32, (8, GW), 1) // Dh
        diag = row == blk

        def body(r, carry):
            g = r // NC
            c = r % NC
            slot = r % S

            @pl.when(c == 0)
            def _():
                wait_all(wq_v.at[g], wq_sem.at[g])
                x8 = jnp.broadcast_to(x_v[0], (8, D))
                q = jnp.dot(x8, wq_v[g], preferred_element_type=f32)
                q_s[...] = jnp.where(diag, q, 0.0).astype(bf16)
                m_s[...] = jnp.full(m_s.shape, -jnp.inf, f32)
                l_s[...] = jnp.zeros_like(l_s)
                acc_s[...] = jnp.zeros_like(acc_s)

            wait_all(kv.at[slot], kv_sem.at[slot])

            @pl.when(r + G < NR)
            def _():
                issue_round(r + G)

            @pl.when(r + G == NR)
            def _():
                bounds = (0,) + WD_SPLIT
                for pi in range(len(WD_SPLIT)):
                    for i in range(bounds[pi] // WR, bounds[pi + 1] // WR):
                        rows_dma(wd_hbm, wd_v, i, misc_sem.at[4 + pi], i % 2)

            if compute:
                q = q_s[...]
                s = lax.dot_general(q[:, 0:Dh], kv[slot, 0, 0], NT, preferred_element_type=f32)
                for j in range(1, NH):
                    s = s + lax.dot_general(q[:, j * Dh:(j + 1) * Dh], kv[slot, 0, j], NT, preferred_element_type=f32)
                s = s * scale
                m_old = m_s[...]
                m_new = jnp.maximum(m_old, jnp.max(s, axis=-1, keepdims=True))
                p = jnp.exp(s - m_new[:, :1])
                alpha = jnp.exp(m_old - m_new)
                psum = p[:, 0:128]
                for t in range(1, CR // 128):
                    psum = psum + p[:, t * 128:(t + 1) * 128]
                l_s[...] = alpha * l_s[...] + psum
                pb = p.astype(bf16)
                for j in range(NH):
                    acc_s[:, j * Dh:(j + 1) * Dh] = alpha * acc_s[:, j * Dh:(j + 1) * Dh] + jnp.dot(pb, kv[slot, 1, j], preferred_element_type=f32)
                m_s[...] = m_new

            @pl.when(c == NC - 1)
            def _():
                wait_all(wo_v.at[g], wo_sem.at[g])
                l = jnp.sum(l_s[...], axis=-1, keepdims=True)
                o = jnp.where(diag, acc_s[...] / l, 0.0).astype(bf16)
                out_s[...] += jnp.dot(o, wo_v[g], preferred_element_type=f32)

            @pl.when(r == FFN_AT)
            def _():
                wait_all(wg_v, misc_sem.at[2])
                wait_all(wu_v, misc_sem.at[3])
                x8 = jnp.broadcast_to(x_v[0], (8, D))
                gt = lax.dot_general(x8, wg_v[...], NT, preferred_element_type=f32)
                u = lax.dot_general(x8, wu_v[...], NT, preferred_element_type=f32)
                hid_s[...] = ((gt * jax.nn.sigmoid(gt)) * u).astype(bf16)
            return carry

        lax.fori_loop(0, NR, body, 0)

        cg.wait()
        xf = x_v[0].astype(f32)
        gwf = gw_v[...].astype(f32)
        z = xf[:, 0:128] * gwf[0:1, :]
        for i in range(1, D // 128):
            z = z + xf[:, i * 128:(i + 1) * 128] * gwf[i:i + 1, :]
        gate = jax.nn.sigmoid(jnp.sum(z, axis=-1, keepdims=True))
        a = jnp.sum(out_s[...], axis=0, keepdims=True)
        bounds = (0,) + WD_SPLIT
        b = None
        for pi in range(len(WD_SPLIT)):
            lo, hi = bounds[pi], bounds[pi + 1]
            wait_all(wd_v.at[pl.ds(lo, hi - lo)], misc_sem.at[4 + pi])
            part = jnp.dot(hid_s[:, lo:hi], wd_v[lo:hi, :], preferred_element_type=f32)
            b = part if b is None else b + part
        res = gate * a + (1.0 - gate) * b[0:1]
        o_ref[0] = res.astype(o_ref.dtype)

    any_spec = pl.BlockSpec(memory_space=pl.ANY)
    return pl.pallas_call(
        kernel,
        in_specs=[any_spec] * 9,
        out_specs=pl.BlockSpec(memory_space=pltpu.VMEM),
        out_shape=jax.ShapeDtypeStruct((B, Sq, D), A_x.dtype),
        scratch_shapes=[
            pltpu.VMEM((S, 2, NH, CR, Dh), bf16),
            pltpu.VMEM((1, 1, D), bf16),
            pltpu.VMEM((D // 128, 128), bf16),
            pltpu.VMEM((NG, D, GW), bf16),
            pltpu.VMEM((NG, GW, D), bf16),
            pltpu.VMEM((F, D), bf16),
            pltpu.VMEM((F, D), bf16),
            pltpu.VMEM((F, D), bf16),
            pltpu.VMEM((8, GW), bf16),
            pltpu.VMEM((8, 128), f32),
            pltpu.VMEM((8, 128), f32),
            pltpu.VMEM((8, GW), f32),
            pltpu.VMEM((8, D), f32),
            pltpu.VMEM((8, F), bf16),
            pltpu.SemaphoreType.DMA((S,)),
            pltpu.SemaphoreType.DMA((NG,)),
            pltpu.SemaphoreType.DMA((NG,)),
            pltpu.SemaphoreType.DMA((4 + len(WD_SPLIT),)),
        ],
        compiler_params=pltpu.CompilerParams(vmem_limit_bytes=100 * 1024 * 1024, disable_bounds_checks=nobc),
    )(A_x, gate_w.reshape(D // 128, 128), A_k_cache, A_v_cache, A_wq, A_wo, B_w_gate.T, B_w_up.T, B_w_down)
  return kernel_fn

_impl = build()

@jax.jit
def pallas_gated_mix__sliding_block_cached__swiglu_ffn__decode_kernel(
    A_x, A_k_cache, A_v_cache, A_wq, A_wo, B_x, B_w_gate, B_w_up, B_w_down, gate_w):
    return _impl(A_x, A_k_cache, A_v_cache, A_wq, A_wo, B_x, B_w_gate, B_w_up, B_w_down, gate_w)
```

```python
import functools
import jax
import jax.numpy as jnp
from jax import lax
import jax.experimental.pallas as pl
import jax.experimental.pallas.tpu as pltpu

def build(NH=4, ROWS=32, CR=512, G=3, nobc=False, WD_SPLIT=(0, 1024, 1280, 1376), compute=True, wpos=(3, 8, 13), PRE=5, pro_prio='1'):
  def kernel_fn(A_x, A_k_cache, A_v_cache, A_wq, A_wo, B_x, B_w_gate, B_w_up, B_w_down, gate_w):
    B, Sq, D = A_x.shape
    H, Sk, Dh = A_k_cache.shape[1], A_k_cache.shape[2], A_k_cache.shape[3]
    F = B_w_gate.shape[1]
    W = min(4096, max(256, Sk // 4))
    scale = Dh ** -0.5
    NC = W // CR
    NG = H // NH
    NR = NG * NC
    ND = CR // ROWS
    S = G + 1
    GW = NH * Dh
    WR = 32
    NWQ = D // WR
    NWO = GW // WR
    assert NWQ == 2 * NC and NWO == 2 * NC
    NF = F // WR
    NFR = NF - PRE
    assert F % WR == 0 and D == GW
    assert G < NR - 1 and max(wpos) < ND and NFR + 3 < NR - 1
    assert WD_SPLIT[0] == 0 and WD_SPLIT[-1] == F and all(b % WR == 0 for b in WD_SPLIT)
    NP = len(WD_SPLIT) - 1
    PRO_SEM = S - 1
    WD_SEM = [(NR - 1 - G) % S] + [S + i for i in range(NP - 1)]
    NSEM = S + NP - 1
    f32, bf16 = jnp.float32, jnp.bfloat16
    NT = (((1,), (1,)), ((), ()))

    def kernel(x_hbm, gw_hbm, k_hbm, v_hbm, wq_hbm, wo_hbm, wg_hbm, wu_hbm, wd_hbm, o_ref,
               kv, x_v, gw_v, wq_v, wo_v, wg_v, wu_v, wd_v, q_s, m_s, l_s, acc_s, out_s, gt_s, hid_s, gate_s,
               sem):
        def kv_dma(r, which, j):
            g = r // NC
            c = r % NC
            slot = r % S
            src = (k_hbm, v_hbm)[which]
            return pltpu.make_async_copy(
                src.at[0, pl.ds(g * NH, NH), pl.ds(Sk - W + c * CR + j * ROWS, ROWS), :],
                kv.at[slot, which, :, pl.ds(j * ROWS, ROWS), :], sem.at[slot])

        def wq_dma(g, i, s):
            return pltpu.make_async_copy(wq_hbm.at[pl.ds(i * WR, WR), pl.ds(g * GW, GW)],
                                         wq_v.at[g, pl.ds(i * WR, WR), :], sem.at[s])

        def wo_dma(g, i, s):
            return pltpu.make_async_copy(wo_hbm.at[pl.ds(g * GW + i * WR, WR), :],
                                         wo_v.at[g, pl.ds(i * WR, WR), :], sem.at[s])

        def rows_dma(src, dst, i, s):
            return pltpu.make_async_copy(src.at[pl.ds(i * WR, WR), :], dst.at[pl.ds(i * WR, WR), :], sem.at[s])

        def issue_round(r):
            g = r // NC
            c = r % NC
            slot = r % S
            for j in range(ND):
                kv_dma(r, 0, j).start(priority=0)
                kv_dma(r, 1, j).start(priority=1)
                if j == wpos[0]:
                    wo_dma(g, 2 * c, slot).start(priority=0)
                    wo_dma(g, 2 * c + 1, slot).start(priority=1)
                if j == wpos[1]:
                    @pl.when(g + 1 < NG)
                    def _():
                        wq_dma(g + 1, 2 * c, slot).start(priority=0)
                        wq_dma(g + 1, 2 * c + 1, slot).start(priority=1)
                if j == wpos[2]:
                    @pl.when(r < NFR)
                    def _():
                        rows_dma(wg_hbm, wg_v, r + PRE, slot).start(priority=0)
                        rows_dma(wu_hbm, wu_v, r + PRE, slot).start(priority=1)

        def wait_all(buf, s):
            pltpu.make_async_copy(buf, buf, sem.at[s]).wait()

        def wait_round(r):
            g = r // NC
            c = r % NC
            slot = r % S
            wait_all(kv.at[slot], slot)
            wo_dma(g, 2 * c, slot).wait()
            wo_dma(g, 2 * c + 1, slot).wait()

            @pl.when(g + 1 < NG)
            def _():
                wq_dma(g + 1, 2 * c, slot).wait()
                wq_dma(g + 1, 2 * c + 1, slot).wait()

            @pl.when(r < NFR)
            def _():
                rows_dma(wg_hbm, wg_v, r + PRE, slot).wait()
                rows_dma(wu_hbm, wu_v, r + PRE, slot).wait()

        pro = [pltpu.make_async_copy(x_hbm, x_v, sem.at[PRO_SEM]), pltpu.make_async_copy(gw_hbm, gw_v, sem.at[PRO_SEM])]
        pro += [wq_dma(0, i, PRO_SEM) for i in range(NWQ)]
        for i in range(PRE):
            pro += [rows_dma(wg_hbm, wg_v, i, PRO_SEM), rows_dma(wu_hbm, wu_v, i, PRO_SEM)]
        for n, d in enumerate(pro):
            d.start(priority=0 if n < 2 else int(pro_prio[n % len(pro_prio)]))

        def pro_body(r, carry):
            issue_round(r)
            return carry
        lax.fori_loop(0, G, pro_body, 0)

        for d in pro:
            d.wait()
        out_s[...] = jnp.zeros_like(out_s)
        row = lax.broadcasted_iota(jnp.int32, (8, GW), 0)
        blk = lax.broadcasted_iota(jnp.int32, (8, GW), 1) // Dh
        diag = row == blk

        xf = x_v[0].astype(f32)
        gwf = gw_v[...].astype(f32)
        z = xf[:, 0:128] * gwf[0:1, :]
        for i in range(1, D // 128):
            z = z + xf[:, i * 128:(i + 1) * 128] * gwf[i:i + 1, :]
        gate_s[...] = jnp.broadcast_to(jax.nn.sigmoid(jnp.sum(z, axis=-1, keepdims=True)), gate_s.shape)

        def body(r, carry):
            g = r // NC
            c = r % NC
            slot = r % S

            @pl.when(c == 0)
            def _():
                x8 = jnp.broadcast_to(x_v[0], (8, D))
                q = jnp.dot(x8, wq_v[g], preferred_element_type=f32)
                q_s[...] = jnp.where(diag, q, 0.0).astype(bf16)
                m_s[...] = jnp.full(m_s.shape, -jnp.inf, f32)
                l_s[...] = jnp.zeros_like(l_s)
                acc_s[...] = jnp.zeros_like(acc_s)

            wait_round(r)

            @pl.when(r + G < NR - 1)
            def _():
                issue_round(r + G)

            @pl.when(r + G == NR - 1)
            def _():
                rl = NR - 1
                hi = [kv_dma(rl, 0, j) for j in range(ND)]
                hi += [wo_dma(NG - 1, NWO - 2, rl % S), wo_dma(NG - 1, NWO - 1, rl % S)]
                hi += [kv_dma(rl, 1, j) for j in range(ND)]
                lo = []
                for pi in range(NP):
                    for i in range(WD_SPLIT[pi] // WR, WD_SPLIT[pi + 1] // WR):
                        lo.append(rows_dma(wd_hbm, wd_v, i, WD_SEM[pi]))
                assert len(lo) >= len(hi)
                for n, d in enumerate(lo):
                    if n < len(hi):
                        hi[n].start(priority=0)
                    d.start(priority=1)

            if compute:
                q = q_s[...]
                s = lax.dot_general(q[:, 0:Dh], kv[slot, 0, 0], NT, preferred_element_type=f32)
                for j in range(1, NH):
                    s = s + lax.dot_general(q[:, j * Dh:(j + 1) * Dh], kv[slot, 0, j], NT, preferred_element_type=f32)
                s = s * scale
                m_old = m_s[...]
                m_new = jnp.maximum(m_old, jnp.max(s, axis=-1, keepdims=True))
                p = jnp.exp(s - m_new[:, :1])
                alpha = jnp.exp(m_old - m_new)
                psum = p[:, 0:128]
                for t in range(1, CR // 128):
                    psum = psum + p[:, t * 128:(t + 1) * 128]
                l_s[...] = alpha * l_s[...] + psum
                pb = p.astype(bf16)
                for j in range(NH):
                    acc_s[:, j * Dh:(j + 1) * Dh] = alpha * acc_s[:, j * Dh:(j + 1) * Dh] + jnp.dot(pb, kv[slot, 1, j], preferred_element_type=f32)
                m_s[...] = m_new

            @pl.when(c == NC - 1)
            def _():
                l = jnp.sum(l_s[...], axis=-1, keepdims=True)
                o = jnp.where(diag, acc_s[...] / l, 0.0).astype(bf16)
                out_s[...] += jnp.dot(o, wo_v[g], preferred_element_type=f32)

            @pl.when(r == NFR + 1)
            def _():
                x8 = jnp.broadcast_to(x_v[0], (8, D))
                gt = lax.dot_general(x8, wg_v[...], NT, preferred_element_type=f32)
                gt_s[...] = gt * jax.nn.sigmoid(gt)

            @pl.when(r == NFR + 3)
            def _():
                x8 = jnp.broadcast_to(x_v[0], (8, D))
                u = lax.dot_general(x8, wu_v[...], NT, preferred_element_type=f32)
                hid_s[...] = (gt_s[...] * u).astype(bf16)
            return carry

        lax.fori_loop(0, NR, body, 0)

        a = jnp.sum(out_s[...], axis=0, keepdims=True)
        out_s[...] = gate_s[...] * a
        for pi in range(NP):
            lo, hi = WD_SPLIT[pi], WD_SPLIT[pi + 1]
            wait_all(wd_v.at[pl.ds(lo, hi - lo)], WD_SEM[pi])
            part = jnp.dot(hid_s[:, lo:hi], wd_v[lo:hi, :], preferred_element_type=f32)
            res = out_s[...] + (1.0 - gate_s[...]) * part
            if pi + 1 < NP:
                out_s[...] = res
            else:
                o_ref[0] = res[0:1].astype(o_ref.dtype)

    any_spec = pl.BlockSpec(memory_space=pl.ANY)
    return pl.pallas_call(
        kernel,
        in_specs=[any_spec] * 9,
        out_specs=pl.BlockSpec(memory_space=pltpu.VMEM),
        out_shape=jax.ShapeDtypeStruct((B, Sq, D), A_x.dtype),
        scratch_shapes=[
            pltpu.VMEM((S, 2, NH, CR, Dh), bf16),
            pltpu.VMEM((1, 1, D), bf16),
            pltpu.VMEM((D // 128, 128), bf16),
            pltpu.VMEM((NG, D, GW), bf16),
            pltpu.VMEM((NG, GW, D), bf16),
            pltpu.VMEM((F, D), bf16),
            pltpu.VMEM((F, D), bf16),
            pltpu.VMEM((F, D), bf16),
            pltpu.VMEM((8, GW), bf16),
            pltpu.VMEM((8, 128), f32),
            pltpu.VMEM((8, 128), f32),
            pltpu.VMEM((8, GW), f32),
            pltpu.VMEM((8, D), f32),
            pltpu.VMEM((8, F), f32),
            pltpu.VMEM((8, F), bf16),
            pltpu.VMEM((8, D), f32),
            pltpu.SemaphoreType.DMA((NSEM,)),
        ],
        compiler_params=pltpu.CompilerParams(vmem_limit_bytes=100 * 1024 * 1024, disable_bounds_checks=nobc),
    )(A_x, gate_w.reshape(D // 128, 128), A_k_cache, A_v_cache, A_wq, A_wo, B_w_gate.T, B_w_up.T, B_w_down)
  return kernel_fn

_impl = build()

@jax.jit
def pallas_gated_mix__sliding_block_cached__swiglu_ffn__decode_kernel(
    A_x, A_k_cache, A_v_cache, A_wq, A_wo, B_x, B_w_gate, B_w_up, B_w_down, gate_w):
    return _impl(A_x, A_k_cache, A_v_cache, A_wq, A_wo, B_x, B_w_gate, B_w_up, B_w_down, gate_w)
```

```python
import jax
import jax.numpy as jnp
from jax import lax
import jax.experimental.pallas as pl
import jax.experimental.pallas.tpu as pltpu

NH = 4
CR = 512
ROWS = 32
WR = 32
AHEAD = 3
WPOS = (3, 8, 13)
PRE = 5
HI, LO = 0, 1


@jax.jit
def pallas_gated_mix__sliding_block_cached__swiglu_ffn__decode_kernel(
    A_x: jax.Array,
    A_k_cache: jax.Array,
    A_v_cache: jax.Array,
    A_wq: jax.Array,
    A_wo: jax.Array,
    B_x: jax.Array,
    B_w_gate: jax.Array,
    B_w_up: jax.Array,
    B_w_down: jax.Array,
    gate_w: jax.Array,
):
    del B_x
    B, Sq, D = A_x.shape
    _, H, Sk, Dh = A_k_cache.shape
    F = B_w_gate.shape[1]
    W = min(4096, max(256, Sk // 4))
    scale = Dh ** -0.5
    f32, bf16 = jnp.float32, jnp.bfloat16

    NC = W // CR
    NG = H // NH
    NR = NG * NC
    ND = CR // ROWS
    S = AHEAD + 1
    GW = NH * Dh
    NW = 2 * NC
    QR = D // NH // NW
    NFR = F // WR - PRE
    WD = (0, 1024, F - 128, F)
    NP = len(WD) - 1
    assert (B, Sq) == (1, 1) and Dh == 128 and D == GW and GW == NW * WR and QR == 8
    assert W % CR == 0 and H % NH == 0 and F % WR == 0 and all(b % WR == 0 for b in WD)
    assert NFR + 3 < NR - 1 - AHEAD and F // WR >= 2 * ND + 2
    PRO_SEM, OUT_SEM, WD_SEM = S, S + 1, S + 2
    NT = (((1,), (1,)), ((), ()))

    def kernel(x_hbm, gw_hbm, k_hbm, v_hbm, wq_hbm, wo_hbm, wg_hbm, wu_hbm, wd_hbm, o_hbm,
               kv, x_v, gw_v, wq_v, wo_v, wg_v, wu_v, wd_v,
               q_s, m_s, l_s, acc_s, out_s, gt_s, hid_s, gate_s, hcol_s, res_v):

        def main(sem):
            def kv_dma(r, which, j):
                src = (k_hbm, v_hbm)[which]
                row0 = Sk - W + (r % NC) * CR + j * ROWS
                return pltpu.make_async_copy(
                    src.at[0, pl.ds((r // NC) * NH, NH), pl.ds(row0, ROWS), :],
                    kv.at[r % S, which, :, pl.ds(j * ROWS, ROWS), :], sem.at[r % S])

            def wq_dma(g, i, s):
                return pltpu.make_async_copy(wq_hbm.at[:, pl.ds(i * QR, QR), pl.ds(g * GW, GW)],
                                             wq_v.at[g, :, pl.ds(i * QR, QR), :], sem.at[s])

            def wo_dma(g, i, s):
                return pltpu.make_async_copy(wo_hbm.at[pl.ds(g * GW + i * WR, WR), :],
                                             wo_v.at[g, pl.ds(i * WR, WR), :], sem.at[s])

            def rows_dma(src, dst, i, s):
                return pltpu.make_async_copy(src.at[pl.ds(i * WR, WR), :],
                                             dst.at[pl.ds(i * WR, WR), :], sem.at[s])

            def wait_all(buf, s):
                pltpu.make_async_copy(buf, buf, sem.at[s]).wait()

            def wo_pair(r):
                return [wo_dma(r // NC, 2 * (r % NC) + i, r % S) for i in range(2)]

            def wq_pair(r):
                return [wq_dma(r // NC + 1, 2 * (r % NC) + i, r % S) for i in range(2)]

            def ffn_pair(r):
                return [rows_dma(wg_hbm, wg_v, r + PRE, r % S), rows_dma(wu_hbm, wu_v, r + PRE, r % S)]

            def start_pair(pair):
                pair[0].start(priority=HI)
                pair[1].start(priority=LO)

            def wait_pair(pair):
                pair[0].wait()
                pair[1].wait()

            def issue_round(r):
                for j in range(ND):
                    start_pair([kv_dma(r, 0, j), kv_dma(r, 1, j)])
                    if j == WPOS[0]:
                        start_pair(wo_pair(r))
                    if j == WPOS[1]:
                        pl.when(r // NC + 1 < NG)(lambda: start_pair(wq_pair(r)))
                    if j == WPOS[2]:
                        pl.when(r < NFR)(lambda: start_pair(ffn_pair(r)))

            def issue_last_round():
                rl = NR - 1
                hi = [kv_dma(rl, 0, j) for j in range(ND)] + wo_pair(rl) + [kv_dma(rl, 1, j) for j in range(ND)]
                n = 0
                for p in range(NP):
                    for i in range(WD[p] // WR, WD[p + 1] // WR):
                        if n < len(hi):
                            hi[n].start(priority=HI)
                        rows_dma(wd_hbm, wd_v, i, WD_SEM + p).start(priority=LO)
                        n += 1

            def wait_round(r):
                wait_all(kv.at[r % S], r % S)
                wait_pair(wo_pair(r))
                pl.when(r // NC + 1 < NG)(lambda: wait_pair(wq_pair(r)))
                pl.when(r < NFR)(lambda: wait_pair(ffn_pair(r)))

            pro = [wq_dma(0, i, PRO_SEM) for i in range(NW)]
            for i in range(PRE):
                pro += [rows_dma(wg_hbm, wg_v, i, PRO_SEM), rows_dma(wu_hbm, wu_v, i, PRO_SEM)]
            tiny = [pltpu.make_async_copy(x_hbm, x_v, sem.at[PRO_SEM]),
                    pltpu.make_async_copy(gw_hbm, gw_v, sem.at[PRO_SEM])]
            for d in pro:
                d.start(priority=LO)
            for d in tiny:
                d.start(priority=HI)

            def fill(r, carry):
                issue_round(r)
                return carry
            lax.fori_loop(0, AHEAD, fill, 0)

            for d in pro + tiny:
                d.wait()

            out_s[...] = jnp.zeros_like(out_s)
            diag = (lax.broadcasted_iota(jnp.int32, (8, GW), 0)
                    == lax.broadcasted_iota(jnp.int32, (8, GW), 1) // Dh)
            xf = x_v[0].astype(f32)
            gwf = gw_v[...].astype(f32)
            z = xf[:, 0:128] * gwf[0:1, :]
            for i in range(1, D // 128):
                z = z + xf[:, i * 128:(i + 1) * 128] * gwf[i:i + 1, :]
            gate_s[...] = jnp.broadcast_to(jax.nn.sigmoid(jnp.sum(z, axis=-1, keepdims=True)), gate_s.shape)

            def body(r, carry):
                g = r // NC
                c = r % NC
                slot = r % S

                @pl.when(c == 0)
                def _():
                    x8 = jnp.broadcast_to(x_v[0], (8, D))
                    q = jnp.dot(x8, wq_v[g].reshape(D, GW), preferred_element_type=f32)
                    q_s[...] = jnp.where(diag, q, 0.0).astype(bf16)
                    m_s[...] = jnp.full(m_s.shape, -jnp.inf, f32)
                    l_s[...] = jnp.zeros_like(l_s)
                    acc_s[...] = jnp.zeros_like(acc_s)

                wait_round(r)
                pl.when(r + AHEAD < NR - 1)(lambda: issue_round(r + AHEAD))
                pl.when(r + AHEAD == NR - 1)(issue_last_round)

                q = q_s[...]
                s = lax.dot_general(q[:, 0:Dh], kv[slot, 0, 0], NT, preferred_element_type=f32)
                for j in range(1, NH):
                    s = s + lax.dot_general(q[:, j * Dh:(j + 1) * Dh], kv[slot, 0, j], NT,
                                            preferred_element_type=f32)
                s = s * scale
                m_old = m_s[...]
                m_new = jnp.maximum(m_old, jnp.max(s, axis=-1, keepdims=True))
                p = jnp.exp(s - m_new[:, :1])
                alpha = jnp.exp(m_old - m_new)
                psum = p[:, 0:128]
                for t in range(1, CR // 128):
                    psum = psum + p[:, t * 128:(t + 1) * 128]
                l_s[...] = alpha * l_s[...] + psum
                pb = p.astype(bf16)
                for j in range(NH):
                    cols = slice(j * Dh, (j + 1) * Dh)
                    acc_s[:, cols] = alpha * acc_s[:, cols] + jnp.dot(pb, kv[slot, 1, j],
                                                                      preferred_element_type=f32)
                m_s[...] = m_new

                @pl.when(c == NC - 1)
                def _():
                    l = jnp.sum(l_s[...], axis=-1, keepdims=True)
                    o = jnp.where(diag, acc_s[...] / l, 0.0).astype(bf16)
                    out_s[...] += jnp.dot(o, wo_v[g], preferred_element_type=f32)

                @pl.when(r == NFR + 1)
                def _():
                    x8 = jnp.broadcast_to(x_v[0], (8, D))
                    gt = lax.dot_general(x8, wg_v[...], NT, preferred_element_type=f32)
                    gt_s[...] = gt * jax.nn.sigmoid(gt)

                @pl.when(r == NFR + 3)
                def _():
                    x8 = jnp.broadcast_to(x_v[0], (8, D))
                    u = lax.dot_general(x8, wu_v[...], NT, preferred_element_type=f32)
                    hid = (gt_s[...] * u).astype(bf16)
                    hid_s[...] = hid
                    eye = (lax.broadcasted_iota(jnp.int32, (128, 128), 0)
                           == lax.broadcasted_iota(jnp.int32, (128, 128), 1))
                    hrow = jnp.broadcast_to(hid[0:1, F - 128:F], (128, 128)).astype(f32)
                    hd = jnp.where(eye, hrow, 0.0).astype(bf16)
                    hc = jnp.dot(hd, jnp.ones((128, 128), bf16), preferred_element_type=f32)
                    hcol_s[...] = hc * (1.0 - gate_s[0:1, 0:128])
                return carry

            lax.fori_loop(0, NR, body, 0)

            sub0 = lax.broadcasted_iota(jnp.int32, (8, D), 0) == 0
            out_s[...] = gate_s[...] * out_s[...]
            for p in range(NP - 1):
                lo, hi = WD[p], WD[p + 1]
                wait_all(wd_v.at[pl.ds(lo, hi - lo)], WD_SEM + p)
                part = jnp.dot(hid_s[:, lo:hi], wd_v[lo:hi, :], preferred_element_type=f32)
                out_s[...] += jnp.where(sub0, (1.0 - gate_s[...]) * part, 0.0)

            lo = WD[NP - 1]
            wait_all(wd_v.at[pl.ds(lo, F - lo)], WD_SEM + NP - 1)
            res = out_s[...]
            for r0 in range(0, F - lo, 16):
                w16 = wd_v[lo + r0:lo + r0 + 16, :].astype(f32)
                for t in range(0, 16, 8):
                    hc = hcol_s[r0 + t:r0 + t + 8, :]
                    res = res + jnp.concatenate([hc] * (D // 128), axis=1) * w16[t:t + 8, :]
            res_v[0] = jnp.sum(res, axis=0, keepdims=True).astype(res_v.dtype)
            out_dma = pltpu.make_async_copy(res_v, o_hbm, sem.at[OUT_SEM])
            out_dma.start()
            out_dma.wait()

        pl.run_scoped(main, pltpu.SemaphoreType.DMA((WD_SEM + NP,)))

    any_spec = pl.BlockSpec(memory_space=pl.ANY)
    return pl.pallas_call(
        kernel,
        in_specs=[any_spec] * 9,
        out_specs=any_spec,
        out_shape=jax.ShapeDtypeStruct((B, Sq, D), A_x.dtype),
        scratch_shapes=[
            pltpu.VMEM((S, 2, NH, CR, Dh), bf16),
            pltpu.VMEM((1, 1, D), bf16),
            pltpu.VMEM((D // 128, 128), bf16),
            pltpu.VMEM((NG, NH, D // NH, GW), bf16),
            pltpu.VMEM((NG, GW, D), bf16),
            pltpu.VMEM((F, D), bf16),
            pltpu.VMEM((F, D), bf16),
            pltpu.VMEM((F, D), bf16),
            pltpu.VMEM((8, GW), bf16),
            pltpu.VMEM((8, 128), f32),
            pltpu.VMEM((8, 128), f32),
            pltpu.VMEM((8, GW), f32),
            pltpu.VMEM((8, D), f32),
            pltpu.VMEM((8, F), f32),
            pltpu.VMEM((8, F), bf16),
            pltpu.VMEM((8, D), f32),
            pltpu.VMEM((128, 128), f32),
            pltpu.VMEM((1, 1, D), bf16),
        ],
        compiler_params=pltpu.CompilerParams(vmem_limit_bytes=64 * 1024 * 1024),
    )(A_x, gate_w.reshape(D // 128, 128), A_k_cache, A_v_cache, A_wq.reshape(NH, D // NH, H * Dh),
      A_wo, B_w_gate.T, B_w_up.T, B_w_down)
```

```python
import jax
import jax.numpy as jnp
from jax import lax
import jax.experimental.pallas as pl
import jax.experimental.pallas.tpu as pltpu

NH = 4
CR = 512
ROWS = 32
WR = 32
AHEAD = 3
WPOS = 11
PRE = 5
HI, LO = 0, 1


@jax.jit
def pallas_gated_mix__sliding_block_cached__swiglu_ffn__decode_kernel(
    A_x: jax.Array,
    A_k_cache: jax.Array,
    A_v_cache: jax.Array,
    A_wq: jax.Array,
    A_wo: jax.Array,
    B_x: jax.Array,
    B_w_gate: jax.Array,
    B_w_up: jax.Array,
    B_w_down: jax.Array,
    gate_w: jax.Array,
):
    del B_x
    B, Sq, D = A_x.shape
    _, H, Sk, Dh = A_k_cache.shape
    F = B_w_gate.shape[1]
    W = min(4096, max(256, Sk // 4))
    scale = Dh ** -0.5
    f32, bf16 = jnp.float32, jnp.bfloat16

    NC = W // CR
    NG = H // NH
    NR = NG * NC
    ND = CR // ROWS
    S = AHEAD + 1
    GW = NH * Dh
    NW = 2 * NC
    QR = D // NH // NW
    NFR = F // WR - PRE
    WD = (0, 1024, F - 128, F)
    NP = len(WD) - 1
    assert (B, Sq) == (1, 1) and Dh == 128 and D == GW and GW == NW * WR and QR == 8
    assert W % CR == 0 and H % NH == 0 and F % WR == 0 and all(b % WR == 0 for b in WD)
    assert NFR + 3 < NR - 1 - AHEAD and F // WR >= 2 * ND + 2 and WPOS < ND
    PRO_SEM, OUT_SEM, WD_SEM = S, S + 1, S + 2
    NT = (((1,), (1,)), ((), ()))

    def kernel(x_hbm, gw_hbm, k_hbm, v_hbm, wq_hbm, wo_hbm, wg_hbm, wu_hbm, wd_hbm, o_hbm,
               kv, x_v, gw_v, wq_v, wo_v, wg_v, wu_v, wd_v,
               q_s, m_s, l_s, acc_s, out_s, gt_s, hid_s, gate_s, hcol_s, res_v):

        def main(sem):
            def kv_dma(r, which, j):
                src = (k_hbm, v_hbm)[which]
                row0 = Sk - W + (r % NC) * CR + j * ROWS
                return pltpu.make_async_copy(
                    src.at[0, pl.ds((r // NC) * NH, NH), pl.ds(row0, ROWS), :],
                    kv.at[r % S, which, :, pl.ds(j * ROWS, ROWS), :], sem.at[r % S])

            def wq_dma(g, i, s):
                return pltpu.make_async_copy(wq_hbm.at[:, pl.ds(i * QR, QR), pl.ds(g * GW, GW)],
                                             wq_v.at[g, :, pl.ds(i * QR, QR), :], sem.at[s])

            def wo_dma(g, i, s):
                return pltpu.make_async_copy(wo_hbm.at[pl.ds(g * GW + i * WR, WR), :],
                                             wo_v.at[g, pl.ds(i * WR, WR), :], sem.at[s])

            def rows_dma(src, dst, i, s):
                return pltpu.make_async_copy(src.at[pl.ds(i * WR, WR), :],
                                             dst.at[pl.ds(i * WR, WR), :], sem.at[s])

            def wait_all(buf, s):
                pltpu.make_async_copy(buf, buf, sem.at[s]).wait()

            def wo_pair(r):
                return [wo_dma(r // NC, 2 * (r % NC) + i, r % S) for i in range(2)]

            def wq_pair(r):
                return [wq_dma(r // NC + 1, 2 * (r % NC) + i, r % S) for i in range(2)]

            def ffn_pair(r):
                return [rows_dma(wg_hbm, wg_v, r + PRE, r % S), rows_dma(wu_hbm, wu_v, r + PRE, r % S)]

            def start_pair(pair):
                pair[0].start(priority=HI)
                pair[1].start(priority=LO)

            def wait_pair(pair):
                pair[0].wait()
                pair[1].wait()

            def issue_round(r):
                for j in range(ND):
                    start_pair([kv_dma(r, 0, j), kv_dma(r, 1, j)])
                    if j == WPOS:
                        start_pair(wo_pair(r))
                        pl.when(r // NC + 1 < NG)(lambda: start_pair(wq_pair(r)))
                        pl.when(r < NFR)(lambda: start_pair(ffn_pair(r)))

            def issue_last_round():
                rl = NR - 1
                hi = [kv_dma(rl, 0, j) for j in range(ND)] + wo_pair(rl) + [kv_dma(rl, 1, j) for j in range(ND)]
                n = 0
                for p in range(NP):
                    for i in range(WD[p] // WR, WD[p + 1] // WR):
                        if n < len(hi):
                            hi[n].start(priority=HI)
                        rows_dma(wd_hbm, wd_v, i, WD_SEM + p).start(priority=LO)
                        n += 1

            def wait_round(r):
                wait_all(kv.at[r % S], r % S)
                wait_pair(wo_pair(r))
                pl.when(r // NC + 1 < NG)(lambda: wait_pair(wq_pair(r)))
                pl.when(r < NFR)(lambda: wait_pair(ffn_pair(r)))

            pro = [wq_dma(0, i, PRO_SEM) for i in range(NW)]
            for i in range(PRE):
                pro += [rows_dma(wg_hbm, wg_v, i, PRO_SEM), rows_dma(wu_hbm, wu_v, i, PRO_SEM)]
            tiny = [pltpu.make_async_copy(x_hbm, x_v, sem.at[PRO_SEM]),
                    pltpu.make_async_copy(gw_hbm, gw_v, sem.at[PRO_SEM])]
            for d in pro:
                d.start(priority=LO)
            for d in tiny:
                d.start(priority=HI)

            def fill(r, carry):
                issue_round(r)
                return carry
            lax.fori_loop(0, AHEAD, fill, 0)

            for d in pro + tiny:
                d.wait()

            out_s[...] = jnp.zeros_like(out_s)
            diag = (lax.broadcasted_iota(jnp.int32, (8, GW), 0)
                    == lax.broadcasted_iota(jnp.int32, (8, GW), 1) // Dh)
            xf = x_v[0].astype(f32)
            gwf = gw_v[...].astype(f32)
            z = xf[:, 0:128] * gwf[0:1, :]
            for i in range(1, D // 128):
                z = z + xf[:, i * 128:(i + 1) * 128] * gwf[i:i + 1, :]
            gate_s[...] = jnp.broadcast_to(jax.nn.sigmoid(jnp.sum(z, axis=-1, keepdims=True)), gate_s.shape)

            def body(r, carry):
                g = r // NC
                c = r % NC
                slot = r % S

                @pl.when(c == 0)
                def _():
                    x8 = jnp.broadcast_to(x_v[0], (8, D))
                    q = jnp.dot(x8, wq_v[g].reshape(D, GW), preferred_element_type=f32)
                    q_s[...] = jnp.where(diag, q, 0.0).astype(bf16)
                    m_s[...] = jnp.full(m_s.shape, -jnp.inf, f32)
                    l_s[...] = jnp.zeros_like(l_s)
                    acc_s[...] = jnp.zeros_like(acc_s)

                wait_round(r)
                pl.when(r + AHEAD < NR - 1)(lambda: issue_round(r + AHEAD))
                pl.when(r + AHEAD == NR - 1)(issue_last_round)

                q = q_s[...]
                s = lax.dot_general(q[:, 0:Dh], kv[slot, 0, 0], NT, preferred_element_type=f32)
                for j in range(1, NH):
                    s = s + lax.dot_general(q[:, j * Dh:(j + 1) * Dh], kv[slot, 0, j], NT,
                                            preferred_element_type=f32)
                s = s * scale
                m_old = m_s[...]
                m_new = jnp.maximum(m_old, jnp.max(s, axis=-1, keepdims=True))
                p = jnp.exp(s - m_new[:, :1])
                alpha = jnp.exp(m_old - m_new)
                psum = p[:, 0:128]
                for t in range(1, CR // 128):
                    psum = psum + p[:, t * 128:(t + 1) * 128]
                l_s[...] = alpha * l_s[...] + psum
                pb = p.astype(bf16)
                for j in range(NH):
                    cols = slice(j * Dh, (j + 1) * Dh)
                    acc_s[:, cols] = alpha * acc_s[:, cols] + jnp.dot(pb, kv[slot, 1, j],
                                                                      preferred_element_type=f32)
                m_s[...] = m_new

                @pl.when(c == NC - 1)
                def _():
                    l = jnp.sum(l_s[...], axis=-1, keepdims=True)
                    o = jnp.where(diag, acc_s[...] / l, 0.0).astype(bf16)
                    out_s[...] += jnp.dot(o, wo_v[g], preferred_element_type=f32)

                @pl.when(r == NFR + 1)
                def _():
                    x8 = jnp.broadcast_to(x_v[0], (8, D))
                    gt = lax.dot_general(x8, wg_v[...], NT, preferred_element_type=f32)
                    gt_s[...] = gt * jax.nn.sigmoid(gt)

                @pl.when(r == NFR + 3)
                def _():
                    x8 = jnp.broadcast_to(x_v[0], (8, D))
                    u = lax.dot_general(x8, wu_v[...], NT, preferred_element_type=f32)
                    hid = (gt_s[...] * u).astype(bf16)
                    hid_s[...] = hid
                    eye = (lax.broadcasted_iota(jnp.int32, (128, 128), 0)
                           == lax.broadcasted_iota(jnp.int32, (128, 128), 1))
                    hrow = jnp.broadcast_to(hid[0:1, F - 128:F], (128, 128)).astype(f32)
                    hd = jnp.where(eye, hrow, 0.0).astype(bf16)
                    hc = jnp.dot(hd, jnp.ones((128, 128), bf16), preferred_element_type=f32)
                    hcol_s[...] = hc * (1.0 - gate_s[0:1, 0:128])
                return carry

            lax.fori_loop(0, NR, body, 0)

            sub0 = lax.broadcasted_iota(jnp.int32, (8, D), 0) == 0
            out_s[...] = gate_s[...] * out_s[...]
            for p in range(NP - 1):
                lo, hi = WD[p], WD[p + 1]
                wait_all(wd_v.at[pl.ds(lo, hi - lo)], WD_SEM + p)
                part = jnp.dot(hid_s[:, lo:hi], wd_v[lo:hi, :], preferred_element_type=f32)
                out_s[...] += jnp.where(sub0, (1.0 - gate_s[...]) * part, 0.0)

            lo = WD[NP - 1]
            wait_all(wd_v.at[pl.ds(lo, F - lo)], WD_SEM + NP - 1)
            res = out_s[...]
            for r0 in range(0, F - lo, 16):
                w16 = wd_v[lo + r0:lo + r0 + 16, :].astype(f32)
                for t in range(0, 16, 8):
                    hc = hcol_s[r0 + t:r0 + t + 8, :]
                    res = res + jnp.concatenate([hc] * (D // 128), axis=1) * w16[t:t + 8, :]
            res_v[0] = jnp.sum(res, axis=0, keepdims=True).astype(res_v.dtype)
            out_dma = pltpu.make_async_copy(res_v, o_hbm, sem.at[OUT_SEM])
            out_dma.start()
            out_dma.wait()

        pl.run_scoped(main, pltpu.SemaphoreType.DMA((WD_SEM + NP,)))

    any_spec = pl.BlockSpec(memory_space=pl.ANY)
    return pl.pallas_call(
        kernel,
        in_specs=[any_spec] * 9,
        out_specs=any_spec,
        out_shape=jax.ShapeDtypeStruct((B, Sq, D), A_x.dtype),
        scratch_shapes=[
            pltpu.VMEM((S, 2, NH, CR, Dh), bf16),
            pltpu.VMEM((1, 1, D), bf16),
            pltpu.VMEM((D // 128, 128), bf16),
            pltpu.VMEM((NG, NH, D // NH, GW), bf16),
            pltpu.VMEM((NG, GW, D), bf16),
            pltpu.VMEM((F, D), bf16),
            pltpu.VMEM((F, D), bf16),
            pltpu.VMEM((F, D), bf16),
            pltpu.VMEM((8, GW), bf16),
            pltpu.VMEM((8, 128), f32),
            pltpu.VMEM((8, 128), f32),
            pltpu.VMEM((8, GW), f32),
            pltpu.VMEM((8, D), f32),
            pltpu.VMEM((8, F), f32),
            pltpu.VMEM((8, F), bf16),
            pltpu.VMEM((8, D), f32),
            pltpu.VMEM((128, 128), f32),
            pltpu.VMEM((1, 1, D), bf16),
        ],
        compiler_params=pltpu.CompilerParams(vmem_limit_bytes=64 * 1024 * 1024),
    )(A_x, gate_w.reshape(D // 128, 128), A_k_cache, A_v_cache, A_wq.reshape(NH, D // NH, H * Dh),
      A_wo, B_w_gate.T, B_w_up.T, B_w_down)
```

```python
import jax
import jax.numpy as jnp
from jax import lax
import jax.experimental.pallas as pl
import jax.experimental.pallas.tpu as pltpu

NH = 4
CR = 512
ROWS = 32
WR = 32
AHEAD = 3
WPOS = 11
PRE = 5
HI, LO = 0, 1


@jax.jit
def pallas_gated_mix__sliding_block_cached__swiglu_ffn__decode_kernel(
    A_x: jax.Array,
    A_k_cache: jax.Array,
    A_v_cache: jax.Array,
    A_wq: jax.Array,
    A_wo: jax.Array,
    B_x: jax.Array,
    B_w_gate: jax.Array,
    B_w_up: jax.Array,
    B_w_down: jax.Array,
    gate_w: jax.Array,
):
    del B_x
    B, Sq, D = A_x.shape
    _, H, Sk, Dh = A_k_cache.shape
    F = B_w_gate.shape[1]
    W = min(4096, max(256, Sk // 4))
    scale = Dh ** -0.5
    f32, bf16 = jnp.float32, jnp.bfloat16

    NC = W // CR
    NG = H // NH
    NR = NG * NC
    ND = CR // ROWS
    S = AHEAD + 1
    GW = NH * Dh
    NW = 2 * NC
    QR = D // NH // NW
    NFR = F // WR - PRE
    WD = (0, 1024, F - 128, F - WR, F)
    NP, NVP = len(WD) - 1, 2
    assert (B, Sq) == (1, 1) and Dh == 128 and D == GW and GW == NW * WR and QR == 8
    assert W % CR == 0 and H % NH == 0 and F % WR == 0 and all(b % WR == 0 for b in WD)
    assert NFR + 3 < NR - 1 - AHEAD and F // WR >= 2 * ND + 2 and WPOS < ND
    PRO_SEM, OUT_SEM, WD_SEM = S, S + 1, S + 2
    NT = (((1,), (1,)), ((), ()))

    def kernel(x_hbm, gw_hbm, k_hbm, v_hbm, wq_hbm, wo_hbm, wg_hbm, wu_hbm, wd_hbm, o_hbm,
               kv, x_v, gw_v, wq_v, wo_v, wg_v, wu_v, wd_v,
               q_s, m_s, l_s, acc_s, out_s, gt_s, hid_s, gate_s, hcol_s, res_v):

        def main(sem):
            def kv_dma(r, which, j):
                src = (k_hbm, v_hbm)[which]
                row0 = Sk - W + (r % NC) * CR + j * ROWS
                return pltpu.make_async_copy(
                    src.at[0, pl.ds((r // NC) * NH, NH), pl.ds(row0, ROWS), :],
                    kv.at[r % S, which, :, pl.ds(j * ROWS, ROWS), :], sem.at[r % S])

            def wq_dma(g, i, s):
                return pltpu.make_async_copy(wq_hbm.at[:, pl.ds(i * QR, QR), pl.ds(g * GW, GW)],
                                             wq_v.at[g, :, pl.ds(i * QR, QR), :], sem.at[s])

            def wo_dma(g, i, s):
                return pltpu.make_async_copy(wo_hbm.at[pl.ds(g * GW + i * WR, WR), :],
                                             wo_v.at[g, pl.ds(i * WR, WR), :], sem.at[s])

            def rows_dma(src, dst, i, s):
                return pltpu.make_async_copy(src.at[pl.ds(i * WR, WR), :],
                                             dst.at[pl.ds(i * WR, WR), :], sem.at[s])

            def wait_all(buf, s):
                pltpu.make_async_copy(buf, buf, sem.at[s]).wait()

            def wo_pair(r):
                return [wo_dma(r // NC, 2 * (r % NC) + i, r % S) for i in range(2)]

            def wq_pair(r):
                return [wq_dma(r // NC + 1, 2 * (r % NC) + i, r % S) for i in range(2)]

            def ffn_pair(r):
                return [rows_dma(wg_hbm, wg_v, r + PRE, r % S), rows_dma(wu_hbm, wu_v, r + PRE, r % S)]

            def start_pair(pair):
                pair[0].start(priority=HI)
                pair[1].start(priority=LO)

            def wait_pair(pair):
                pair[0].wait()
                pair[1].wait()

            def issue_round(r):
                for j in range(ND):
                    start_pair([kv_dma(r, 0, j), kv_dma(r, 1, j)])
                    if j == WPOS:
                        start_pair(wo_pair(r))
                        pl.when(r // NC + 1 < NG)(lambda: start_pair(wq_pair(r)))
                        pl.when(r < NFR)(lambda: start_pair(ffn_pair(r)))

            def issue_last_round():
                rl = NR - 1
                hi = [kv_dma(rl, 0, j) for j in range(ND)] + wo_pair(rl) + [kv_dma(rl, 1, j) for j in range(ND)]
                n = 0
                for p in range(NP):
                    for i in range(WD[p] // WR, WD[p + 1] // WR):
                        if n < len(hi):
                            hi[n].start(priority=HI)
                        rows_dma(wd_hbm, wd_v, i, WD_SEM + p).start(priority=LO)
                        n += 1

            def wait_round(r):
                for j in range(ND):
                    wait_pair([kv_dma(r, 0, j), kv_dma(r, 1, j)])
                wait_pair(wo_pair(r))
                pl.when(r // NC + 1 < NG)(lambda: wait_pair(wq_pair(r)))
                pl.when(r < NFR)(lambda: wait_pair(ffn_pair(r)))

            pro = [wq_dma(0, i, PRO_SEM) for i in range(NW)]
            for i in range(PRE):
                pro += [rows_dma(wg_hbm, wg_v, i, PRO_SEM), rows_dma(wu_hbm, wu_v, i, PRO_SEM)]
            tiny = [pltpu.make_async_copy(x_hbm, x_v, sem.at[PRO_SEM]),
                    pltpu.make_async_copy(gw_hbm, gw_v, sem.at[PRO_SEM])]
            for d in pro:
                d.start(priority=LO)
            for d in tiny:
                d.start(priority=HI)

            def fill(r, carry):
                issue_round(r)
                return carry
            lax.fori_loop(0, AHEAD, fill, 0)

            for d in pro + tiny:
                d.wait()

            out_s[...] = jnp.zeros_like(out_s)
            diag = (lax.broadcasted_iota(jnp.int32, (8, GW), 0)
                    == lax.broadcasted_iota(jnp.int32, (8, GW), 1) // Dh)
            xf = x_v[0].astype(f32)
            gwf = gw_v[...].astype(f32)
            z = xf[:, 0:128] * gwf[0:1, :]
            for i in range(1, D // 128):
                z = z + xf[:, i * 128:(i + 1) * 128] * gwf[i:i + 1, :]
            gate_s[...] = jnp.broadcast_to(jax.nn.sigmoid(jnp.sum(z, axis=-1, keepdims=True)), gate_s.shape)

            def body(r, carry):
                g = r // NC
                c = r % NC
                slot = r % S

                @pl.when(c == 0)
                def _():
                    x8 = jnp.broadcast_to(x_v[0], (8, D))
                    q = jnp.dot(x8, wq_v[g].reshape(D, GW), preferred_element_type=f32)
                    q_s[...] = jnp.where(diag, q, 0.0).astype(bf16)
                    m_s[...] = jnp.full(m_s.shape, -jnp.inf, f32)
                    l_s[...] = jnp.zeros_like(l_s)
                    acc_s[...] = jnp.zeros_like(acc_s)

                wait_round(r)
                pl.when(r + AHEAD < NR - 1)(lambda: issue_round(r + AHEAD))
                pl.when(r + AHEAD == NR - 1)(issue_last_round)

                q = q_s[...]
                s = lax.dot_general(q[:, 0:Dh], kv[slot, 0, 0], NT, preferred_element_type=f32)
                for j in range(1, NH):
                    s = s + lax.dot_general(q[:, j * Dh:(j + 1) * Dh], kv[slot, 0, j], NT,
                                            preferred_element_type=f32)
                s = s * scale
                m_old = m_s[...]
                m_new = jnp.maximum(m_old, jnp.max(s, axis=-1, keepdims=True))
                p = jnp.exp(s - m_new[:, :1])
                alpha = jnp.exp(m_old - m_new)
                psum = p[:, 0:128]
                for t in range(1, CR // 128):
                    psum = psum + p[:, t * 128:(t + 1) * 128]
                l_s[...] = alpha * l_s[...] + psum
                pb = p.astype(bf16)
                for j in range(NH):
                    cols = slice(j * Dh, (j + 1) * Dh)
                    acc_s[:, cols] = alpha * acc_s[:, cols] + jnp.dot(pb, kv[slot, 1, j],
                                                                      preferred_element_type=f32)
                m_s[...] = m_new

                @pl.when(c == NC - 1)
                def _():
                    l = jnp.sum(l_s[...], axis=-1, keepdims=True)
                    o = jnp.where(diag, acc_s[...] / l, 0.0).astype(bf16)
                    out_s[...] += jnp.dot(o, wo_v[g], preferred_element_type=f32)

                @pl.when(r == NFR + 1)
                def _():
                    x8 = jnp.broadcast_to(x_v[0], (8, D))
                    gt = lax.dot_general(x8, wg_v[...], NT, preferred_element_type=f32)
                    gt_s[...] = gt * jax.nn.sigmoid(gt)

                @pl.when(r == NFR + 3)
                def _():
                    x8 = jnp.broadcast_to(x_v[0], (8, D))
                    u = lax.dot_general(x8, wu_v[...], NT, preferred_element_type=f32)
                    hid = (gt_s[...] * u).astype(bf16)
                    hid_s[...] = hid
                    eye = (lax.broadcasted_iota(jnp.int32, (128, 128), 0)
                           == lax.broadcasted_iota(jnp.int32, (128, 128), 1))
                    hrow = jnp.broadcast_to(hid[0:1, F - 128:F], (128, 128)).astype(f32)
                    hd = jnp.where(eye, hrow, 0.0).astype(bf16)
                    hc = jnp.dot(hd, jnp.ones((128, 128), bf16), preferred_element_type=f32)
                    hcol_s[...] = hc * (1.0 - gate_s[0:1, 0:128])
                return carry

            lax.fori_loop(0, NR, body, 0)

            sub0 = lax.broadcasted_iota(jnp.int32, (8, D), 0) == 0
            out_s[...] = gate_s[...] * out_s[...]
            for p in range(NP):
                lo, hi = WD[p], WD[p + 1]
                wait_all(wd_v.at[pl.ds(lo, hi - lo)], WD_SEM + p)
                res = out_s[...]
                if p < NP - NVP:
                    part = jnp.dot(hid_s[:, lo:hi], wd_v[lo:hi, :], preferred_element_type=f32)
                    res = res + jnp.where(sub0, (1.0 - gate_s[...]) * part, 0.0)
                else:
                    for r0 in range(lo, hi, 16):
                        w16 = wd_v[r0:r0 + 16, :].astype(f32)
                        for t in range(0, 16, 8):
                            h0 = r0 + t - (F - 128)
                            hc = jnp.concatenate([hcol_s[h0:h0 + 8, :]] * (D // 128), axis=1)
                            res = res + hc * w16[t:t + 8, :]
                if p + 1 < NP:
                    out_s[...] = res
                else:
                    res_v[0] = jnp.sum(res, axis=0, keepdims=True).astype(res_v.dtype)
            out_dma = pltpu.make_async_copy(res_v, o_hbm, sem.at[OUT_SEM])
            out_dma.start()
            out_dma.wait()

        pl.run_scoped(main, pltpu.SemaphoreType.DMA((WD_SEM + NP,)))

    any_spec = pl.BlockSpec(memory_space=pl.ANY)
    return pl.pallas_call(
        kernel,
        in_specs=[any_spec] * 9,
        out_specs=any_spec,
        out_shape=jax.ShapeDtypeStruct((B, Sq, D), A_x.dtype),
        scratch_shapes=[
            pltpu.VMEM((S, 2, NH, CR, Dh), bf16),
            pltpu.VMEM((1, 1, D), bf16),
            pltpu.VMEM((D // 128, 128), bf16),
            pltpu.VMEM((NG, NH, D // NH, GW), bf16),
            pltpu.VMEM((NG, GW, D), bf16),
            pltpu.VMEM((F, D), bf16),
            pltpu.VMEM((F, D), bf16),
            pltpu.VMEM((F, D), bf16),
            pltpu.VMEM((8, GW), bf16),
            pltpu.VMEM((8, 128), f32),
            pltpu.VMEM((8, 128), f32),
            pltpu.VMEM((8, GW), f32),
            pltpu.VMEM((8, D), f32),
            pltpu.VMEM((8, F), f32),
            pltpu.VMEM((8, F), bf16),
            pltpu.VMEM((8, D), f32),
            pltpu.VMEM((128, 128), f32),
            pltpu.VMEM((1, 1, D), bf16),
        ],
        compiler_params=pltpu.CompilerParams(vmem_limit_bytes=64 * 1024 * 1024),
    )(A_x, gate_w.reshape(D // 128, 128), A_k_cache, A_v_cache, A_wq.reshape(NH, D // NH, H * Dh),
      A_wo, B_w_gate.T, B_w_up.T, B_w_down)
```
